```python
import jax
import jax.numpy as jnp

def _softmax(x, axis=-1):
    return jax.nn.softmax(x, axis=axis)
def _gelu(x):
    return jax.nn.gelu(x, approximate=True)
def _silu(x):
    return jax.nn.silu(x)
def _sigmoid(x):
    return jax.nn.sigmoid(x)
def _layernorm(x, axis=-1, eps=1e-5):
    m = jnp.mean(x, axis=axis, keepdims=True)
    v = jnp.var(x, axis=axis, keepdims=True)
    return (x - m) / jnp.sqrt(v + eps)
def _scatter_add(tgt, idx, src, axis=0):
    return tgt.at[idx].add(src)
def _segment_sum(src, seg, n):
    return jax.ops.segment_sum(src, seg, n)
class _Rng:
    def __init__(self, key):
        self._k = key
    def _next(self):
        self._k, sub = jax.random.split(self._k)
        return sub
    def normal(self, shape):
        return jax.random.normal(self._next(), shape, dtype=jnp.bfloat16)
    def randint(self, lo, hi, shape):
        return jax.random.randint(self._next(), shape, lo, hi, dtype=jnp.int32)
    def uniform(self, shape, lo=0.0, hi=1.0):
        return jax.random.uniform(self._next(), shape, jnp.bfloat16, lo, hi)
    def permutation(self, n):
        return jax.random.permutation(self._next(), n)


kernel_name = 'parallel_sum__sliding_block_cached__mixer_s_mlp__decode'

def setup_inputs():
    _rng = _Rng(jax.random.key(int.from_bytes(__import__("os").urandom(4), "little")))
    _w = (lambda a: (lambda t: t.astype(jnp.bfloat16) if jnp.issubdtype(t.dtype, jnp.floating) else t)(jnp.asarray(a)))
    def _A_setup():
        B, Sq, D = 4, 1, 512
        Hq, Hkv, Sk, Dh = 32, 32, 8192, 128
        assert Hq % Hkv == 0, (Hq, Hkv)
        return {
            "x": _w((lambda *s: _rng.normal(s) * 0.05)(B, Sq, D)),
            "k_cache": _w((lambda *s: _rng.normal(s) * 0.05)(B, Hkv, Sk, Dh)),
            "v_cache": _w((lambda *s: _rng.normal(s) * 0.05)(B, Hkv, Sk, Dh)),
            "wq": _w((lambda *s: _rng.normal(s) * 0.05)(D, Hq * Dh) * (D ** -0.5)),
            "wo": _w((lambda *s: _rng.normal(s) * 0.05)(Hq * Dh, D) * ((Hq * Dh) ** -0.5)),
        }
    _A_in = _A_setup()

    def _B_setup():
        B, S, D, F = 4, 1, 512, 1376
        return {
            "x":  _w((lambda *s: _rng.normal(s) * 0.05)(B, S, D)),
            "w1": _w((lambda *s: _rng.normal(s) * 0.05)(D, D) * (D ** -0.5)),
            "w2": _w((lambda *s: _rng.normal(s) * 0.05)(D, D) * (D ** -0.5)),
            "w3": _w((lambda *s: _rng.normal(s) * 0.05)(D, F) * (D ** -0.5)),
            "w4": _w((lambda *s: _rng.normal(s) * 0.05)(F, D) * (F ** -0.5)),
        }
    _B_in = _B_setup()

    return {
        "A_x": _A_in["x"],
        "A_k_cache": _A_in["k_cache"],
        "A_v_cache": _A_in["v_cache"],
        "A_wq": _A_in["wq"],
        "A_wo": _A_in["wo"],
        "B_x": _B_in["x"],
        "B_w1": _B_in["w1"],
        "B_w2": _B_in["w2"],
        "B_w3": _B_in["w3"],
        "B_w4": _B_in["w4"],
    }

def reference(A_x, A_k_cache, A_v_cache, A_wq, A_wo, B_x, B_w1, B_w2, B_w3, B_w4):
    def _A_ref(x, k_cache, v_cache, wq, wo):
        B, Sq, D = x.shape
        Hq, Dh = 32, 128
        Hkv, Sk = k_cache.shape[1], k_cache.shape[2]
        W = min(4096, max(256, Sk // 4))
        rep = Hq // Hkv
        q = (lambda x, *d: x.transpose(*d))((x @ wq).reshape(B, Sq, Hq, Dh), 0, 2, 1, 3)
        k = jnp.repeat(k_cache[:, :, Sk - W:, :], rep, axis=1)
        v = jnp.repeat(v_cache[:, :, Sk - W:, :], rep, axis=1)
        scores = jnp.einsum("bhqd,bhkd->bhqk", q, k) * (Dh ** -0.5)
        p = _softmax(scores, axis=-1)
        o = jnp.einsum("bhqk,bhkd->bhqd", p, v)
        return (lambda x, *d: x.transpose(*d))(o, 0, 2, 1, 3).reshape(B, Sq, Hq * Dh) @ wo

    def _B_ref(x, w1, w2, w3, w4):
        B, S, D = x.shape
        h = _gelu(_layernorm(x, axis=-1) @ w1)
        c = D // 4
        g0 = jnp.pad(h[:, :, 0*c:1*c], ((0, 0), (1, 0), (0, 0)))[:, :S, :]
        g1 = jnp.pad(h[:, :, 1*c:2*c], ((0, 0), (0, 1), (0, 0)))[:, 1:, :]
        g2 = jnp.pad(h[:, :, 2*c:3*c], ((0, 0), (2, 0), (0, 0)))[:, :S, :]
        g3 = jnp.pad(h[:, :, 3*c:   ], ((0, 0), (0, 2), (0, 0)))[:, 2:, :]
        hs = jnp.concatenate([g0, g1, g2, g3], axis=-1) @ w2
        x1 = x + hs
        h2 = _gelu(_layernorm(x1, axis=-1) @ w3) @ w4
        return x1 + h2

    x = A_x
    xn = _layernorm(x, axis=-1)
    return x + _A_ref(xn, A_k_cache, A_v_cache, A_wq, A_wo) + _B_ref(xn, B_w1, B_w2, B_w3, B_w4)
```

```python
import jax, jax.numpy as jnp, functools
from jax import lax
import jax.experimental.pallas as pl
import jax.experimental.pallas.tpu as pltpu

B, D, H, SK, DH, F = 4, 512, 32, 8192, 128, 1376
W = 2048
HB = 8
NG = B * H // HB
CH = 256
NC = W // CH
PR = 16
ND = CH // PR
L = 4
SCALE = DH ** -0.5
BF = jnp.bfloat16
F32 = jnp.float32


def _ln(x, eps=1e-5):
    m = jnp.mean(x, axis=-1, keepdims=True)
    xc = x - m
    v = jnp.mean(xc * xc, axis=-1, keepdims=True)
    return xc / jnp.sqrt(v + eps)


def kernel(x_hbm, k_hbm, v_hbm, wq_hbm, wo_hbm, w3_hbm, w4_hbm, o_ref,
           kbuf, vbuf, wq_v, wo_v, w3_v, w4_v, x_v, q2, o2, s_scr, p_scr, linv, oacc, lhs, acc, xn_scr,
           sem0, sem1, wsem):
    def kv_desc(hbm, buf, grp, c, r, slot, sem):
        g = grp // B
        b = grp % B
        row = c * CH + r * PR
        return pltpu.make_async_copy(
            hbm.at[b, pl.ds(g * HB, HB), pl.ds(SK - W + row, PR), :],
            buf.at[slot, :, pl.ds(row, PR), :], sem)

    def wq_desc(c, r):
        g = c // 2
        row = (c % 2) * 256 + r * 16
        sem = wsem.at[jnp.minimum(g, 1)] if not isinstance(c, int) else wsem.at[min(g, 1)]
        return pltpu.make_async_copy(wq_hbm.at[pl.ds(row, 16), pl.ds(g * 1024, 1024)],
                                     wq_v.at[pl.ds(row, 16), pl.ds(g * 1024, 1024)], sem)

    def wo_desc(c, r):
        row = c * 512 + r * 32
        return pltpu.make_async_copy(wo_hbm.at[pl.ds(row, 32), :], wo_v.at[pl.ds(row, 32), :], wsem.at[2])

    def issue_k_wq(t):
        c = t % NC
        for r in range(ND):
            kv_desc(k_hbm, kbuf, 0, c, r, 0, sem0.at[c]).start(priority=0)
            wq_desc(c, r).start(priority=1)

    def issue_k_wo(t):
        c = t % NC
        for r in range(ND):
            kv_desc(k_hbm, kbuf, 1, c, r, 1, sem0.at[c]).start(priority=0)
            wo_desc(c, r).start(priority=1)

    def issue_kv(t):
        c = t % NC
        grp = t // NC
        slot = grp % 2
        for r in range(ND):
            kv_desc(k_hbm, kbuf, grp, c, r, slot, sem0.at[c]).start(priority=0)
            kv_desc(v_hbm, vbuf, grp - 2, c, r, slot, sem1.at[c]).start(priority=1)

    def issue_vv(t):
        c = t % NC
        for r in range(ND):
            kv_desc(v_hbm, vbuf, NG - 1, c, r, 1, sem0.at[c]).start(priority=0)
            kv_desc(v_hbm, vbuf, NG - 2, c, r, 0, sem1.at[c]).start(priority=1)

    def issue_mlp(lo, n):
        for r in range(n):
            row = (lo + r) * 32
            pltpu.make_async_copy(w3_hbm.at[pl.ds(row, 32), :], w3_v.at[pl.ds(row, 32), :], wsem.at[3]).start(priority=0)
            pltpu.make_async_copy(w4_hbm.at[pl.ds(row, 32), :], w4_v.at[pl.ds(row, 32), :], wsem.at[4]).start(priority=1)

    def wait_unit(buf, slot, c, sem):
        dst = buf.at[slot, :, pl.ds(c * CH, CH), :]
        pltpu.make_async_copy(dst, dst, sem).wait()

    def wait_all(ref, sem):
        pltpu.make_async_copy(ref, ref, sem).wait()

    row8 = lax.broadcasted_iota(jnp.int32, (8, DH), 0)
    row8c = lax.broadcasted_iota(jnp.int32, (8, CH), 0)

    def q_block(g):
        q = jnp.dot(xn_scr[...].astype(BF), wq_v[:, g * 1024:(g + 1) * 1024], preferred_element_type=F32)
        q = q.astype(BF).astype(F32)
        for b in range(B):
            for j in range(HB):
                q2[g * B + b, pl.ds(j, 1), :] = q[b:b + 1, j * DH:(j + 1) * DH]

    def k_phase(u):
        c = u % NC
        grp = u // NC
        slot = grp % 2
        wait_unit(kbuf, slot, c, sem0.at[c])
        qg = q2[grp].astype(BF)
        s = None
        for j in range(HB):
            sj = lax.dot_general(qg, kbuf[slot, j, pl.ds(pl.multiple_of(c * CH, CH), CH), :],
                                 (((1,), (1,)), ((), ())), preferred_element_type=F32)
            s = sj if s is None else jnp.where(row8c == j, sj, s)
        s_scr[c] = s

    def softmax(grp):
        slot = grp % 2
        s = s_scr[...]
        m = jnp.max(jnp.max(s, axis=0), axis=-1, keepdims=True)
        p = jnp.exp((s - m[None]) * SCALE)
        l = jnp.sum(jnp.sum(p, axis=0), axis=-1, keepdims=True)
        p_scr[slot] = p
        linv[slot] = jnp.broadcast_to(1.0 / l, (8, DH))

    def v_compute(grp, c, vslot):
        p = p_scr[grp % 2, c].astype(BF)
        o = None
        for j in range(HB):
            oj = jnp.dot(p, vbuf[vslot, j, pl.ds(pl.multiple_of(c * CH, CH), CH), :], preferred_element_type=F32)
            o = oj if o is None else jnp.where(row8 == j, oj, o)
        return o

    def out_proj(g):
        for b in range(B):
            for j in range(HB):
                lhs[pl.ds(b, 1), j * DH:(j + 1) * DH] = o2[g * B + b, pl.ds(j, 1), :]
        acc[...] += jnp.dot(lhs[...].astype(BF), wo_v[pl.ds(pl.multiple_of(g * 1024, 1024), 1024), :],
                            preferred_element_type=F32)

    xc = pltpu.make_async_copy(x_hbm, x_v, wsem.at[5])
    xc.start(priority=1)
    for t in range(L):
        issue_k_wq(t)
    lhs[...] = jnp.zeros_like(lhs)
    xc.wait()
    x = x_v[...].astype(F32)
    x8 = jnp.concatenate([x, jnp.zeros_like(x)], axis=0)
    xn = _ln(x8)
    xn_scr[...] = xn
    acc[...] = x8 + xn
    wq0 = wq_v.at[:, pl.ds(0, 1024)]
    wait_all(wq0, wsem.at[0])
    q_block(0)

    def loop1(u, carry):
        k_phase(u)
        t = u + L
        @pl.when(t < NC)
        def _(): issue_k_wq(t)
        @pl.when(jnp.logical_and(t >= NC, t < 2 * NC))
        def _(): issue_k_wo(t)
        @pl.when(t >= 2 * NC)
        def _(): issue_kv(t)
        @pl.when(u % NC == NC - 1)
        def _(): softmax(u // NC)
        @pl.when(u == NC - 1)
        def _():
            wait_all(wq_v.at[:, pl.ds(1024, 3072)], wsem.at[1])
            for g in range(1, 4):
                q_block(g)
        return carry
    lax.fori_loop(0, 2 * NC, loop1, 0)

    def loop2(u, carry):
        c = u % NC
        grp = u // NC
        vg = grp - 2
        wait_unit(vbuf, grp % 2, c, sem1.at[c])
        k_phase(u)
        o = v_compute(vg, c, grp % 2)
        oacc[...] = jnp.where(c == 0, o, oacc[...] + o)
        t = u + L
        @pl.when(t < NG * NC)
        def _(): issue_kv(t)
        @pl.when(t >= NG * NC)
        def _(): issue_vv(t)
        @pl.when(c == NC - 1)
        def _():
            o2[vg] = oacc[...] * linv[vg % 2]
            softmax(grp)
            @pl.when(vg % B == B - 1)
            def _():
                @pl.when(vg == B - 1)
                def _(): wait_all(wo_v, wsem.at[2])
                out_proj(vg // B)
        @pl.when(u == 2 * NC + 1)
        def _(): issue_mlp(0, 16)
        @pl.when(u == 3 * NC + 1)
        def _(): issue_mlp(16, 16)
        @pl.when(u == 4 * NC + 1)
        def _(): issue_mlp(32, 11)
        @pl.when(u == 7 * NC + 3)
        def _():
            wait_all(w3_v, wsem.at[3])
            h1 = lax.dot_general(_ln(xn_scr[...]).astype(BF), w3_v[...], (((1,), (1,)), ((), ())), preferred_element_type=F32)
            h1 = jax.nn.gelu(h1, approximate=True)
            wait_all(w4_v, wsem.at[4])
            acc[...] += jnp.dot(h1.astype(BF), w4_v[...], preferred_element_type=F32)
        return carry
    oacc[...] = jnp.zeros_like(oacc)
    lax.fori_loop(2 * NC, NG * NC, loop2, 0)

    def loop3(c, carry):
        oa, ob = carry
        wait_unit(vbuf, 0, c, sem1.at[c])
        wait_unit(vbuf, 1, c, sem0.at[c])
        oa = oa + v_compute(NG - 2, c, 0)
        ob = ob + v_compute(NG - 1, c, 1)
        t = c + L
        @pl.when(t < NC)
        def _(): issue_vv(t)
        return oa, ob
    z = jnp.zeros((8, DH), F32)
    oa, ob = lax.fori_loop(0, NC, loop3, (z, z))
    o2[NG - 2] = oa * linv[0]
    o2[NG - 1] = ob * linv[1]
    out_proj(3)
    o_ref[...] = acc[0:B, :].astype(o_ref.dtype)


@jax.jit
def pallas_parallel_sum__sliding_block_cached__mixer_s_mlp__decode_kernel(A_x, A_k_cache, A_v_cache, A_wq, A_wo, B_x, B_w1, B_w2, B_w3, B_w4):
    any_spec = pl.BlockSpec(memory_space=pl.ANY)
    out = pl.pallas_call(
        kernel,
        in_specs=[any_spec] * 7,
        out_specs=pl.BlockSpec(memory_space=pltpu.VMEM),
        out_shape=jax.ShapeDtypeStruct((B, D), BF),
        scratch_shapes=[
            pltpu.VMEM((2, HB, W, DH), BF),
            pltpu.VMEM((2, HB, W, DH), BF),
            pltpu.VMEM((D, H * DH), BF),
            pltpu.VMEM((H * DH, D), BF),
            pltpu.VMEM((F, D), BF),
            pltpu.VMEM((F, D), BF),
            pltpu.VMEM((B, D), BF),
            pltpu.VMEM((NG, 8, DH), F32),
            pltpu.VMEM((NG, 8, DH), F32),
            pltpu.VMEM((NC, 8, CH), F32),
            pltpu.VMEM((2, NC, 8, CH), F32),
            pltpu.VMEM((2, 8, DH), F32),
            pltpu.VMEM((8, DH), F32),
            pltpu.VMEM((8, 1024), F32),
            pltpu.VMEM((8, D), F32),
            pltpu.VMEM((8, D), F32),
            pltpu.SemaphoreType.DMA((NC,)),
            pltpu.SemaphoreType.DMA((NC,)),
            pltpu.SemaphoreType.DMA((6,)),
        ],
        compiler_params=pltpu.CompilerParams(vmem_limit_bytes=64 * 1024 * 1024),
    )(A_x.reshape(B, D), A_k_cache, A_v_cache, A_wq, A_wo, B_w3.T, B_w4)
    return out.reshape(B, 1, D)
```

```python
import jax
import jax.numpy as jnp
from jax import lax
import jax.experimental.pallas as pl
import jax.experimental.pallas.tpu as pltpu

B, D, H, SK, DH, F = 4, 512, 32, 8192, 128, 1376
W = 2048
HB = 8
NG = B * H // HB
CH = 128
NC = W // CH
PR = 16
ND = CH // PR
L = 10
UPB = NC // 4
N0 = 21
W4_BOUNDS = (12, 19, 21)
SCALE = DH ** -0.5
BF = jnp.bfloat16
F32 = jnp.float32
NT = (((1,), (1,)), ((), ()))

S_X, S_WQ0, S_WQ1, S_WO, S_W3, S_W4 = 0, 1, 2, 3, 4, 5


def _ln(x, eps=1e-5):
    m = jnp.mean(x, axis=-1, keepdims=True)
    xc = x - m
    v = jnp.mean(xc * xc, axis=-1, keepdims=True)
    return xc / jnp.sqrt(v + eps)


def _w4_segs(ci):
    lo = 0 if ci == 0 else W4_BOUNDS[ci - 1]
    hi = W4_BOUNDS[ci]
    hi1 = hi if ci < len(W4_BOUNDS) - 1 else F // 32 - N0
    return (lo * 32, hi * 32), ((N0 + lo) * 32, (N0 + hi1) * 32)


def _kernel(x_hbm, k_hbm, v_hbm, wq_hbm, wo_hbm, w3_hbm, w4_hbm, o_ref,
            kbuf, vbuf, wq_v, wo_v, w3_v, w4_v, x_v,
            q2, o2, s_scr, p_scr, linv, oacc, lhs, acc, xn_scr, hseg,
            sem0, sem1, wsem):
    def kv_desc(hbm, buf, grp, c, r, slot, sem):
        row = c * CH + r * PR
        return pltpu.make_async_copy(
            hbm.at[grp % B, pl.ds((grp // B) * HB, HB), pl.ds(SK - W + row, PR), :],
            buf.at[slot, :, pl.ds(row, PR), :], sem)

    def wq_desc(c, r):
        g = c // UPB
        k = (c % UPB) * ND + r
        sem = wsem.at[S_WQ0 + (min(g, 1) if isinstance(g, int) else jnp.minimum(g, 1))]
        rs, cs = pl.ds((k // 4) * 8, 8), pl.ds(g * 1024 + (k % 4) * 256, 256)
        return pltpu.make_async_copy(wq_hbm.at[:, rs, cs], wq_v.at[:, rs, cs], sem)

    def wo_desc(c, r):
        k = c * ND + r
        rs, cs = pl.ds((k // 2) * 8, 8), pl.ds((k % 2) * 256, 256)
        return pltpu.make_async_copy(wo_hbm.at[:, rs, cs], wo_v.at[:, rs, cs], wsem.at[S_WO])

    def w32(hbm, vm, d, sem):
        rs = pl.ds(d * 32, 32)
        return pltpu.make_async_copy(hbm.at[rs, :], vm.at[rs, :], sem)

    def issue_k_wq(t):
        c = t % NC
        for r in range(ND):
            kv_desc(k_hbm, kbuf, 0, c, r, 0, sem0.at[c]).start(priority=0)
            wq_desc(c, r).start(priority=1)

    def issue_k_wo(t):
        c = t % NC
        for r in range(ND):
            kv_desc(k_hbm, kbuf, 1, c, r, 1, sem0.at[c]).start(priority=0)
            wo_desc(c, r).start(priority=1)

    def issue_kv(t):
        c = t % NC
        grp = t // NC
        slot = grp % 2
        for r in range(ND):
            kv_desc(k_hbm, kbuf, grp, c, r, slot, sem0.at[c]).start(priority=0)
            kv_desc(v_hbm, vbuf, grp - 2, c, r, slot, sem1.at[c]).start(priority=1)

    def issue_vv(t):
        c = t % NC
        for r in range(ND):
            kv_desc(v_hbm, vbuf, NG - 1, c, r, 1, sem0.at[c]).start(priority=0)
            kv_desc(v_hbm, vbuf, NG - 2, c, r, 0, sem1.at[c]).start(priority=1)

    def issue_w3(lo, n, extra=0):
        for r in range(lo, lo + n):
            w32(w3_hbm, w3_v, r, wsem.at[S_W3]).start(priority=0)
            w32(w3_hbm, w3_v, 23 + r, wsem.at[S_W3]).start(priority=1)
        for r in range(extra):
            w32(w3_hbm, w3_v, 20 + r, wsem.at[S_W3]).start(priority=0)

    def issue_w4(ci):
        (a0, b0), (a1, b1) = _w4_segs(ci)
        d0 = list(range(a0 // 32, b0 // 32))
        d1 = list(range(a1 // 32, b1 // 32))
        for r in range(max(len(d0), len(d1))):
            if r < len(d0):
                w32(w4_hbm, w4_v, d0[r], wsem.at[S_W4 + 2 * ci]).start(priority=0)
            if r < len(d1):
                w32(w4_hbm, w4_v, d1[r], wsem.at[S_W4 + 2 * ci + 1]).start(priority=1)

    def wait_region(ref, sem):
        pltpu.make_async_copy(ref, ref, sem).wait()

    def wait_unit(buf, slot, c, sem):
        wait_region(buf.at[slot, :, pl.ds(c * CH, CH), :], sem)

    row_d = lax.broadcasted_iota(jnp.int32, (8, DH), 0)
    row_c = lax.broadcasted_iota(jnp.int32, (8, CH), 0)

    def q_block(g):
        wq_g = wq_v[:, :, g * 1024:(g + 1) * 1024].reshape(D, 1024)
        q = jnp.dot(xn_scr[...].astype(BF), wq_g, preferred_element_type=F32)
        for b in range(B):
            for j in range(HB):
                q2[g * B + b, pl.ds(j, 1), :] = q[b:b + 1, j * DH:(j + 1) * DH]

    def k_phase(u):
        c = u % NC
        grp = u // NC
        slot = grp % 2
        wait_unit(kbuf, slot, c, sem0.at[c])
        qg = q2[grp].astype(BF)
        s = None
        for j in range(HB):
            kj = kbuf[slot, j, pl.ds(pl.multiple_of(c * CH, CH), CH), :]
            sj = lax.dot_general(qg, kj, NT, preferred_element_type=F32)
            s = sj if s is None else jnp.where(row_c == j, sj, s)
        s_scr[c] = s

    def softmax(grp):
        slot = grp % 2
        s = s_scr[...]
        m = jnp.max(jnp.max(s, axis=0), axis=-1, keepdims=True)
        p = jnp.exp((s - m[None]) * SCALE)
        l = jnp.sum(jnp.sum(p, axis=0), axis=-1, keepdims=True)
        p_scr[slot] = p
        linv[slot] = jnp.broadcast_to(1.0 / l, (8, DH))

    def v_compute(grp, c, vslot):
        p = p_scr[grp % 2, c].astype(BF)
        o = None
        for j in range(HB):
            vj = vbuf[vslot, j, pl.ds(pl.multiple_of(c * CH, CH), CH), :]
            oj = jnp.dot(p, vj, preferred_element_type=F32)
            o = oj if o is None else jnp.where(row_d == j, oj, o)
        return o

    def out_proj(g):
        for b in range(B):
            for j in range(HB):
                lhs[pl.ds(b, 1), j * DH:(j + 1) * DH] = o2[g * B + b, pl.ds(j, 1), :]
        wo_g = wo_v[pl.ds(g * 2, 2)].reshape(1024, D)
        acc[...] += jnp.dot(lhs[...].astype(BF), wo_g, preferred_element_type=F32)

    xc = pltpu.make_async_copy(x_hbm, x_v, wsem.at[S_X])
    xc.start(priority=1)
    for t in range(L):
        issue_k_wq(t)
    lhs[...] = jnp.zeros_like(lhs)
    oacc[...] = jnp.zeros_like(oacc)
    xc.wait()
    x = x_v[...].astype(F32)
    x8 = jnp.concatenate([x, jnp.zeros_like(x)], axis=0)
    xn = _ln(x8)
    xn_scr[...] = xn
    acc[...] = x8 + xn
    wait_region(wq_v.at[:, :, pl.ds(0, 1024)], wsem.at[S_WQ0])
    q_block(0)

    def loop1(u, carry):
        k_phase(u)
        t = u + L

        @pl.when(t < NC)
        def _():
            issue_k_wq(t)

        @pl.when(jnp.logical_and(t >= NC, t < 2 * NC))
        def _():
            issue_k_wo(t)

        @pl.when(t >= 2 * NC)
        def _():
            issue_kv(t)

        @pl.when(u % NC == NC - 1)
        def _():
            softmax(u // NC)

        @pl.when(u == NC - 1)
        def _():
            wait_region(wq_v.at[:, :, pl.ds(1024, 3072)], wsem.at[S_WQ1])
            for g in range(1, 4):
                q_block(g)
        return carry

    lax.fori_loop(0, 2 * NC, loop1, 0)

    def loop2(u, carry):
        c = u % NC
        grp = u // NC
        vg = grp - 2
        wait_unit(vbuf, grp % 2, c, sem1.at[c])
        k_phase(u)
        o = v_compute(vg, c, grp % 2)
        oacc[...] = jnp.where(c == 0, o, oacc[...] + o)
        t = u + L

        @pl.when(t < NG * NC)
        def _():
            issue_kv(t)

        @pl.when(t >= NG * NC)
        def _():
            issue_vv(t)

        @pl.when(c == NC - 1)
        def _():
            o2[vg] = oacc[...] * linv[vg % 2]
            softmax(grp)

            @pl.when(vg % B == B - 1)
            def _():
                @pl.when(vg == B - 1)
                def _():
                    wait_region(wo_v, wsem.at[S_WO])
                out_proj(vg // B)

        @pl.when(u == 2 * NC + 1)
        def _():
            issue_w3(0, 8)

        @pl.when(u == 3 * NC + 1)
        def _():
            issue_w3(8, 8)

        @pl.when(u == 4 * NC + 1)
        def _():
            issue_w3(16, 4, extra=3)

        @pl.when(u == 7 * NC + 3)
        def _():
            wait_region(w3_v, wsem.at[S_W3])
            h1 = lax.dot_general(_ln(xn_scr[...]).astype(BF), w3_v[...], NT,
                                 preferred_element_type=F32)
            h1 = jax.nn.gelu(h1, approximate=True)
            for ci in range(len(W4_BOUNDS)):
                for k, (a, b) in enumerate(_w4_segs(ci)):
                    hseg[2 * ci + k, :, 0:b - a] = h1[:, a:b]
        return carry

    lax.fori_loop(2 * NC, NG * NC, loop2, 0)

    def loop3(c, carry):
        oa, ob = carry
        wait_unit(vbuf, 0, c, sem1.at[c])
        wait_unit(vbuf, 1, c, sem0.at[c])
        oa = oa + v_compute(NG - 2, c, 0)
        ob = ob + v_compute(NG - 1, c, 1)
        t = c + L

        @pl.when(t < NC)
        def _():
            issue_vv(t)

        @pl.when(t == NC)
        def _():
            issue_w4(0)

        @pl.when(t == NC + 1)
        def _():
            for ci in range(1, len(W4_BOUNDS)):
                issue_w4(ci)
        return oa, ob

    z = jnp.zeros((8, DH), F32)
    oa, ob = lax.fori_loop(0, NC, loop3, (z, z))
    o2[NG - 2] = oa * linv[0]
    o2[NG - 1] = ob * linv[1]
    out_proj(3)

    y = acc[...]
    for ci in range(len(W4_BOUNDS)):
        for k, (a, b) in enumerate(_w4_segs(ci)):
            wait_region(w4_v.at[pl.ds(a, b - a), :], wsem.at[S_W4 + 2 * ci + k])
        for k, (a, b) in enumerate(_w4_segs(ci)):
            y = y + jnp.dot(hseg[2 * ci + k, :, 0:b - a].astype(BF), w4_v[a:b, :],
                            preferred_element_type=F32)
    o_ref[...] = y[0:B, :].astype(o_ref.dtype)


@jax.jit
def pallas_parallel_sum__sliding_block_cached__mixer_s_mlp__decode_kernel(
        A_x, A_k_cache, A_v_cache, A_wq, A_wo, B_x, B_w1, B_w2, B_w3, B_w4):
    nseg = 2 * len(W4_BOUNDS)
    out = pl.pallas_call(
        _kernel,
        in_specs=[pl.BlockSpec(memory_space=pl.ANY)] * 7,
        out_specs=pl.BlockSpec(memory_space=pltpu.VMEM),
        out_shape=jax.ShapeDtypeStruct((B, D), BF),
        scratch_shapes=[
            pltpu.VMEM((2, HB, W, DH), BF),
            pltpu.VMEM((2, HB, W, DH), BF),
            pltpu.VMEM((8, D // 8, H * DH), BF),
            pltpu.VMEM((8, H * DH // 8, D), BF),
            pltpu.VMEM((F, D), BF),
            pltpu.VMEM((F, D), BF),
            pltpu.VMEM((B, D), BF),
            pltpu.VMEM((NG, 8, DH), F32),
            pltpu.VMEM((NG, 8, DH), F32),
            pltpu.VMEM((NC, 8, CH), F32),
            pltpu.VMEM((2, NC, 8, CH), F32),
            pltpu.VMEM((2, 8, DH), F32),
            pltpu.VMEM((8, DH), F32),
            pltpu.VMEM((8, 1024), F32),
            pltpu.VMEM((8, D), F32),
            pltpu.VMEM((8, D), F32),
            pltpu.VMEM((nseg, 8, 384), F32),
            pltpu.SemaphoreType.DMA((NC,)),
            pltpu.SemaphoreType.DMA((NC,)),
            pltpu.SemaphoreType.DMA((S_W4 + nseg,)),
        ],
        compiler_params=pltpu.CompilerParams(
            vmem_limit_bytes=64 * 1024 * 1024,
            disable_bounds_checks=True,
            disable_semaphore_checks=True),
    )(A_x.reshape(B, D), A_k_cache, A_v_cache,
      A_wq.reshape(8, D // 8, H * DH), A_wo.reshape(8, H * DH // 8, D),
      B_w3.T, B_w4)
    return out.reshape(B, 1, D)
```

```python
import jax
import jax.numpy as jnp
from jax import lax
import jax.experimental.pallas as pl
import jax.experimental.pallas.tpu as pltpu

B, D, H, SK, DH, F = 4, 512, 32, 8192, 128, 1376
W = 2048
HB = 8
NG = B * H // HB
CH = 128
NC = W // CH
PR = 16
ND = CH // PR
L = 10
UPB = NC // 4
W4_BOUNDS = (26, 37, 43)
SCALE = DH ** -0.5
BF = jnp.bfloat16
F32 = jnp.float32
NT = (((1,), (1,)), ((), ()))

S_X, S_WQ0, S_WQ1, S_WO, S_W3, S_W4 = 0, 1, 2, 3, 4, 5


def _ln(x, eps=1e-5):
    m = jnp.mean(x, axis=-1, keepdims=True)
    xc = x - m
    v = jnp.mean(xc * xc, axis=-1, keepdims=True)
    return xc / jnp.sqrt(v + eps)


def _w4_rows(ci):
    lo = 0 if ci == 0 else W4_BOUNDS[ci - 1]
    return lo * 32, W4_BOUNDS[ci] * 32


def _kernel(x_hbm, k_hbm, v_hbm, wq_hbm, wo_hbm, w3_hbm, w4_hbm, o_ref,
            kbuf, vbuf, wq_v, wo_v, w3_v, w4_v, x_v,
            q2, o2, s_scr, p_scr, linv, oacc, lhs, acc, xn_scr, hseg,
            sem0, sem1, wsem):
    def kv_desc(hbm, buf, grp, c, r, slot, sem):
        row = c * CH + r * PR
        return pltpu.make_async_copy(
            hbm.at[grp % B, pl.ds((grp // B) * HB, HB), pl.ds(SK - W + row, PR), :],
            buf.at[slot, :, pl.ds(row, PR), :], sem)

    def wq_desc(c, r):
        g = c // UPB
        k = (c % UPB) * ND + r
        sem = wsem.at[S_WQ0 + (min(g, 1) if isinstance(g, int) else jnp.minimum(g, 1))]
        rs, cs = pl.ds((k // 4) * 8, 8), pl.ds(g * 1024 + (k % 4) * 256, 256)
        return pltpu.make_async_copy(wq_hbm.at[:, rs, cs], wq_v.at[:, rs, cs], sem)

    def wo_desc(c, r):
        k = c * ND + r
        rs, cs = pl.ds((k // 2) * 8, 8), pl.ds((k % 2) * 256, 256)
        return pltpu.make_async_copy(wo_hbm.at[:, rs, cs], wo_v.at[:, rs, cs], wsem.at[S_WO])

    def w32(hbm, vm, d, sem):
        rs = pl.ds(d * 32, 32)
        return pltpu.make_async_copy(hbm.at[rs, :], vm.at[rs, :], sem)

    def issue_k_wq(t):
        c = t % NC
        for r in range(ND):
            kv_desc(k_hbm, kbuf, 0, c, r, 0, sem0.at[c]).start(priority=0)
            wq_desc(c, r).start(priority=1)

    def issue_k_wo(t):
        c = t % NC
        for r in range(ND):
            kv_desc(k_hbm, kbuf, 1, c, r, 1, sem0.at[c]).start(priority=0)
            wo_desc(c, r).start(priority=1)

    def issue_kv(t):
        c = t % NC
        grp = t // NC
        slot = grp % 2
        for r in range(ND):
            kv_desc(k_hbm, kbuf, grp, c, r, slot, sem0.at[c]).start(priority=0)
            kv_desc(v_hbm, vbuf, grp - 2, c, r, slot, sem1.at[c]).start(priority=1)

    def issue_vv(t):
        c = t % NC
        for r in range(ND):
            kv_desc(v_hbm, vbuf, NG - 1, c, r, 1, sem0.at[c]).start(priority=0)
            kv_desc(v_hbm, vbuf, NG - 2, c, r, 0, sem1.at[c]).start(priority=1)

    def issue_w3(lo, n, extra=0):
        for r in range(lo, lo + n):
            w32(w3_hbm, w3_v, r, wsem.at[S_W3]).start(priority=0)
            w32(w3_hbm, w3_v, 23 + r, wsem.at[S_W3]).start(priority=1)
        for r in range(extra):
            w32(w3_hbm, w3_v, 20 + r, wsem.at[S_W3]).start(priority=0)

    def issue_w4(ci):
        a, b = _w4_rows(ci)
        for d in range(a // 32, b // 32):
            w32(w4_hbm, w4_v, d, wsem.at[S_W4 + ci]).start(priority=1)

    def wait_region(ref, sem):
        pltpu.make_async_copy(ref, ref, sem).wait()

    def wait_unit(buf, slot, c, sem):
        wait_region(buf.at[slot, :, pl.ds(c * CH, CH), :], sem)

    row_d = lax.broadcasted_iota(jnp.int32, (8, DH), 0)
    row_c = lax.broadcasted_iota(jnp.int32, (8, CH), 0)

    def q_block(g):
        wq_g = wq_v[:, :, g * 1024:(g + 1) * 1024].reshape(D, 1024)
        q = jnp.dot(xn_scr[...].astype(BF), wq_g, preferred_element_type=F32)
        for b in range(B):
            for j in range(HB):
                q2[g * B + b, pl.ds(j, 1), :] = q[b:b + 1, j * DH:(j + 1) * DH]

    def k_phase(u):
        c = u % NC
        grp = u // NC
        slot = grp % 2
        wait_unit(kbuf, slot, c, sem0.at[c])
        qg = q2[grp].astype(BF)
        s = None
        for j in range(HB):
            kj = kbuf[slot, j, pl.ds(pl.multiple_of(c * CH, CH), CH), :]
            sj = lax.dot_general(qg, kj, NT, preferred_element_type=F32)
            s = sj if s is None else jnp.where(row_c == j, sj, s)
        s_scr[c] = s

    def softmax(grp):
        slot = grp % 2
        s = s_scr[...]
        m = jnp.max(jnp.max(s, axis=0), axis=-1, keepdims=True)
        p = jnp.exp((s - m[None]) * SCALE)
        l = jnp.sum(jnp.sum(p, axis=0), axis=-1, keepdims=True)
        p_scr[slot] = p
        linv[slot] = jnp.broadcast_to(1.0 / l, (8, DH))

    def v_compute(grp, c, vslot):
        p = p_scr[grp % 2, c].astype(BF)
        o = None
        for j in range(HB):
            vj = vbuf[vslot, j, pl.ds(pl.multiple_of(c * CH, CH), CH), :]
            oj = jnp.dot(p, vj, preferred_element_type=F32)
            o = oj if o is None else jnp.where(row_d == j, oj, o)
        return o

    def out_proj(g):
        for b in range(B):
            for j in range(HB):
                lhs[pl.ds(b, 1), j * DH:(j + 1) * DH] = o2[g * B + b, pl.ds(j, 1), :]
        wo_g = wo_v[pl.ds(g * 2, 2)].reshape(1024, D)
        acc[...] += jnp.dot(lhs[...].astype(BF), wo_g, preferred_element_type=F32)

    xc = pltpu.make_async_copy(x_hbm, x_v, wsem.at[S_X])
    xc.start(priority=1)
    for t in range(L):
        issue_k_wq(t)
    lhs[...] = jnp.zeros_like(lhs)
    oacc[...] = jnp.zeros_like(oacc)
    xc.wait()
    x = x_v[...].astype(F32)
    x8 = jnp.concatenate([x, jnp.zeros_like(x)], axis=0)
    xn = _ln(x8)
    xn_scr[...] = xn
    acc[...] = x8 + xn
    wait_region(wq_v.at[:, :, pl.ds(0, 1024)], wsem.at[S_WQ0])
    q_block(0)

    def loop1(u, carry):
        k_phase(u)
        t = u + L

        @pl.when(t < NC)
        def _():
            issue_k_wq(t)

        @pl.when(jnp.logical_and(t >= NC, t < 2 * NC))
        def _():
            issue_k_wo(t)

        @pl.when(t >= 2 * NC)
        def _():
            issue_kv(t)

        @pl.when(u % NC == NC - 1)
        def _():
            softmax(u // NC)

        @pl.when(u == NC - 1)
        def _():
            wait_region(wq_v.at[:, :, pl.ds(1024, 3072)], wsem.at[S_WQ1])
            for g in range(1, 4):
                q_block(g)
        return carry

    lax.fori_loop(0, 2 * NC, loop1, 0)

    def loop2(u, carry):
        c = u % NC
        grp = u // NC
        vg = grp - 2
        wait_unit(vbuf, grp % 2, c, sem1.at[c])
        k_phase(u)
        o = v_compute(vg, c, grp % 2)
        oacc[...] = jnp.where(c == 0, o, oacc[...] + o)
        t = u + L

        @pl.when(t < NG * NC)
        def _():
            issue_kv(t)

        @pl.when(t >= NG * NC)
        def _():
            issue_vv(t)

        @pl.when(c == NC - 1)
        def _():
            o2[vg] = oacc[...] * linv[vg % 2]
            softmax(grp)

            @pl.when(vg % B == B - 1)
            def _():
                @pl.when(vg == B - 1)
                def _():
                    wait_region(wo_v, wsem.at[S_WO])
                out_proj(vg // B)

        @pl.when(u == 2 * NC + 1)
        def _():
            issue_w3(0, 8)

        @pl.when(u == 3 * NC + 1)
        def _():
            issue_w3(8, 8)

        @pl.when(u == 4 * NC + 1)
        def _():
            issue_w3(16, 4, extra=3)

        @pl.when(u == 7 * NC + 3)
        def _():
            wait_region(w3_v, wsem.at[S_W3])
            h1 = lax.dot_general(_ln(xn_scr[...]).astype(BF), w3_v[...], NT,
                                 preferred_element_type=F32)
            h1 = jax.nn.gelu(h1, approximate=True)
            for ci in range(len(W4_BOUNDS)):
                a, b = _w4_rows(ci)
                hseg[ci, :, 0:b - a] = h1[:, a:b]
        return carry

    lax.fori_loop(2 * NC, NG * NC, loop2, 0)

    def loop3(c, carry):
        oa, ob = carry
        wait_unit(vbuf, 0, c, sem1.at[c])
        wait_unit(vbuf, 1, c, sem0.at[c])
        oa = oa + v_compute(NG - 2, c, 0)
        ob = ob + v_compute(NG - 1, c, 1)
        t = c + L

        @pl.when(t < NC)
        def _():
            issue_vv(t)

        @pl.when(t == NC)
        def _():
            issue_w4(0)

        @pl.when(t == NC + 1)
        def _():
            for ci in range(1, len(W4_BOUNDS)):
                issue_w4(ci)
        return oa, ob

    z = jnp.zeros((8, DH), F32)
    oa, ob = lax.fori_loop(0, NC, loop3, (z, z))
    o2[NG - 2] = oa * linv[0]
    o2[NG - 1] = ob * linv[1]
    out_proj(3)

    y = acc[...]
    for ci in range(len(W4_BOUNDS)):
        a, b = _w4_rows(ci)
        wait_region(w4_v.at[pl.ds(a, b - a), :], wsem.at[S_W4 + ci])
        y = y + jnp.dot(hseg[ci, :, 0:b - a].astype(BF), w4_v[a:b, :],
                        preferred_element_type=F32)
    o_ref[...] = y[0:B, :].astype(o_ref.dtype)


@jax.jit
def pallas_parallel_sum__sliding_block_cached__mixer_s_mlp__decode_kernel(
        A_x, A_k_cache, A_v_cache, A_wq, A_wo, B_x, B_w1, B_w2, B_w3, B_w4):
    nseg = len(W4_BOUNDS)
    out = pl.pallas_call(
        _kernel,
        in_specs=[pl.BlockSpec(memory_space=pl.ANY)] * 7,
        out_specs=pl.BlockSpec(memory_space=pltpu.VMEM),
        out_shape=jax.ShapeDtypeStruct((B, D), BF),
        scratch_shapes=[
            pltpu.VMEM((2, HB, W, DH), BF),
            pltpu.VMEM((2, HB, W, DH), BF),
            pltpu.VMEM((8, D // 8, H * DH), BF),
            pltpu.VMEM((8, H * DH // 8, D), BF),
            pltpu.VMEM((F, D), BF),
            pltpu.VMEM((F, D), BF),
            pltpu.VMEM((B, D), BF),
            pltpu.VMEM((NG, 8, DH), F32),
            pltpu.VMEM((NG, 8, DH), F32),
            pltpu.VMEM((NC, 8, CH), F32),
            pltpu.VMEM((2, NC, 8, CH), F32),
            pltpu.VMEM((2, 8, DH), F32),
            pltpu.VMEM((8, DH), F32),
            pltpu.VMEM((8, 1024), F32),
            pltpu.VMEM((8, D), F32),
            pltpu.VMEM((8, D), F32),
            pltpu.VMEM((nseg, 8, 896), F32),
            pltpu.SemaphoreType.DMA((NC,)),
            pltpu.SemaphoreType.DMA((NC,)),
            pltpu.SemaphoreType.DMA((S_W4 + nseg,)),
        ],
        compiler_params=pltpu.CompilerParams(
            vmem_limit_bytes=64 * 1024 * 1024,
            disable_bounds_checks=True,
            disable_semaphore_checks=True),
    )(A_x.reshape(B, D), A_k_cache, A_v_cache,
      A_wq.reshape(8, D // 8, H * DH), A_wo.reshape(8, H * DH // 8, D),
      B_w3.T, B_w4)
    return out.reshape(B, 1, D)
```
